```python
import jax
import jax.numpy as jnp

def _softmax(x, axis=-1):
    return jax.nn.softmax(x, axis=axis)
def _gelu(x):
    return jax.nn.gelu(x, approximate=True)
def _silu(x):
    return jax.nn.silu(x)
def _sigmoid(x):
    return jax.nn.sigmoid(x)
def _layernorm(x, axis=-1, eps=1e-5):
    m = jnp.mean(x, axis=axis, keepdims=True)
    v = jnp.var(x, axis=axis, keepdims=True)
    return (x - m) / jnp.sqrt(v + eps)
def _scatter_add(tgt, idx, src, axis=0):
    return tgt.at[idx].add(src)
def _segment_sum(src, seg, n):
    return jax.ops.segment_sum(src, seg, n)
class _Rng:
    def __init__(self, key):
        self._k = key
    def _next(self):
        self._k, sub = jax.random.split(self._k)
        return sub
    def normal(self, shape):
        return jax.random.normal(self._next(), shape, dtype=jnp.bfloat16)
    def randint(self, lo, hi, shape):
        return jax.random.randint(self._next(), shape, lo, hi, dtype=jnp.int32)
    def uniform(self, shape, lo=0.0, hi=1.0):
        return jax.random.uniform(self._next(), shape, jnp.bfloat16, lo, hi)
    def permutation(self, n):
        return jax.random.permutation(self._next(), n)


kernel_name = 'recurrent_scan__compressed_kv_cla__moe_arch_mod__decode'

def setup_inputs():
    _rng = _Rng(jax.random.key(int.from_bytes(__import__("os").urandom(4), "little")))
    _w = (lambda a: (lambda t: t.astype(jnp.bfloat16) if jnp.issubdtype(t.dtype, jnp.floating) else t)(jnp.asarray(a)))
    def _A_setup():
        B, H, Sq, Sk, D, M = 4, 32, 1, 4096, 128, 576
        Dc = 4 * D
        return {
            "x": _w((lambda *s: _rng.normal(s) * 0.05)(B, Sq, M)),
            "c_kv": _w((lambda *s: _rng.normal(s) * 0.05)(B, Sk, Dc)),
            "w_q": _w((lambda *s: _rng.normal(s) * 0.05)(M, H, D) * (M ** -0.5)),
            "w_uk": _w((lambda *s: _rng.normal(s) * 0.05)(Dc, H, D) * (Dc ** -0.5)),
            "w_uv": _w((lambda *s: _rng.normal(s) * 0.05)(Dc, H, D) * (Dc ** -0.5)),
            "w_o": _w((lambda *s: _rng.normal(s) * 0.05)(H, D, M) * ((H * D) ** -0.5)),
        }
    _A_in = _A_setup()

    def _B_setup():
        B, S, D, F, C = 4, 1, 576, 4608, 1
        return {
            "x": _w((lambda *s: _rng.normal(s) * 0.05)(B, S, D)),
            "w_r": _w((lambda *s: _rng.normal(s) * 0.05)(D)),
            "w_gate": _w((lambda *s: _rng.normal(s) * 0.05)(D, F)),
            "w_up": _w((lambda *s: _rng.normal(s) * 0.05)(D, F)),
            "w_down": _w((lambda *s: _rng.normal(s) * 0.05)(F, D)),
        }
    _B_in = _B_setup()

    return {
        "A_x": _A_in["x"],
        "A_c_kv": _A_in["c_kv"],
        "A_w_q": _A_in["w_q"],
        "A_w_uk": _A_in["w_uk"],
        "A_w_uv": _A_in["w_uv"],
        "A_w_o": _A_in["w_o"],
        "B_x": _B_in["x"],
        "B_w_r": _B_in["w_r"],
        "B_w_gate": _B_in["w_gate"],
        "B_w_up": _B_in["w_up"],
        "B_w_down": _B_in["w_down"],
    }

def reference(A_x, A_c_kv, A_w_q, A_w_uk, A_w_uv, A_w_o, B_x, B_w_r, B_w_gate, B_w_up, B_w_down):
    def _A_ref(x, c_kv, w_q, w_uk, w_uv, w_o):
        B, Sq, M = x.shape[0], x.shape[1], x.shape[2]
        Sk = c_kv.shape[1]
        H, D = w_q.shape[1], w_q.shape[2]
        q = jnp.einsum("bqm,mhd->bhqd", x, w_q)
        k = jnp.einsum("bkc,chd->bhkd", c_kv, w_uk)
        v = jnp.einsum("bkc,chd->bhkd", c_kv, w_uv)
        scores = jnp.einsum("bhqd,bhkd->bhqk", q, k) * (D ** -0.5)
        off = Sk - Sq
        qi = jnp.arange(Sq)[:, None]
        kj = jnp.arange(Sk)[None, :]
        cmask = kj <= (qi + off)
        scores = jnp.where(cmask[None, None], scores, -1e9)
        p = _softmax(scores, axis=-1)
        ctx = jnp.einsum("bhqk,bhkd->bhqd", p, v)
        return jnp.einsum("bhqd,hdm->bqm", ctx, w_o)

    def _B_ref(x, w_r, w_gate, w_up, w_down):
        B, S, D = x.shape
        C = 1
        r = x @ w_r
        idx = jnp.argsort(-r, axis=-1)[:, :C]
        idx_e = jnp.repeat(idx.reshape(B, C, 1), D, axis=2)
        x_sel = jnp.take_along_axis(x, idx_e, axis=1)
        g = _silu(x_sel @ w_gate)
        u = x_sel @ w_up
        y = (g * u) @ w_down
        r_sel = _sigmoid(jnp.take_along_axis(r, idx, axis=1))
        y = y * r_sel.reshape(B, C, 1)
        b_off = (jnp.arange(B) * S).reshape(B, 1)
        flat_idx = (idx + b_off).reshape(B * C)
        zero = (x * 0.0).reshape(B * S, D)
        upd = _scatter_add(zero, flat_idx, y.reshape(B * C, D), axis=0)
        return x + upd.reshape(B, S, D)

    x = A_x
    xn = _layernorm(x, axis=-1)
    s = _A_ref(xn, A_c_kv, A_w_q, A_w_uk, A_w_uv, A_w_o)
    g = _silu(_B_ref(xn, B_w_r, B_w_gate, B_w_up, B_w_down))
    return x + s * g
```

```python
import jax
import jax.numpy as jnp
import numpy as np
from jax import lax
from jax.experimental import pallas as pl
from jax.experimental.pallas import tpu as pltpu

B, M, H, D, DC, SK, F = 4, 576, 32, 128, 512, 4096, 4608
NP = H // 2
BF = jnp.bfloat16
F32 = jnp.float32
NT = (((1,), (1,)), ((), ()))

KC = 512
FC = 512
DCc = 256


def _dot(a, b):
    return jnp.dot(a, b, preferred_element_type=F32)


def _dot_nt(a, b):
    return lax.dot_general(a, b, NT, preferred_element_type=F32)


def _iota(shape, dim):
    return lax.broadcasted_iota(jnp.int32, shape, dim)


def _kernel(x_hbm, wr_hbm, ckv_hbm, wq_hbm, wuk_hbm, wuv_hbm, wo_hbm, wg_hbm, wu_hbm, wd_hbm,
            o_ref,
            x_v, wr_v, ckv_v, wq_v, wuk_v, wuv_v, wo_v, wgu_v, wd_v,
            z_v, row_v, s_v, p_v, h_v, sems):
    wq32 = wq_hbm.bitcast(jnp.uint32)
    wuk32 = wuk_hbm.bitcast(jnp.uint32)
    wuv32 = wuv_hbm.bitcast(jnp.uint32)
    cp = pltpu.make_async_copy

    cp(x_hbm, x_v, sems.at[0]).start()
    cp(wr_hbm, wr_v, sems.at[1]).start()
    for j in range(NP):
        cp(wq32.at[:, j], wq_v.at[j], sems.at[2]).start()
    for j in range(NP):
        cp(wuk32.at[:, j], wuk_v.at[j], sems.at[3]).start(priority=1)
    for b in range(B):
        cp(ckv_hbm.at[b], ckv_v.at[b], sems.at[4 + b]).start(priority=1)
    cp(wo_hbm, wo_v, sems.at[9]).start(priority=1)
    cp(wg_hbm, wgu_v.at[pl.ds(0, M)], sems.at[10]).start(priority=1)
    cp(wu_hbm, wgu_v.at[pl.ds(M, M)], sems.at[10]).start(priority=1)
    cp(wd_hbm.at[:, pl.ds(0, F // 2)], wd_v.at[pl.ds(0, M)], sems.at[11]).start(priority=1)
    cp(wd_hbm.at[:, pl.ds(F // 2, F // 2)], wd_v.at[pl.ds(M, M)], sems.at[11]).start(priority=1)

    exp2 = (_iota((128, 256), 0) == _iota((128, 256), 1) // 2).astype(F32).astype(BF)
    cmp2 = (_iota((256, 128), 0) // 2 == _iota((256, 128), 1)).astype(F32).astype(BF)

    cp(x_hbm, x_v, sems.at[0]).wait()
    cp(wr_hbm, wr_v, sems.at[1]).wait()
    x = x_v[...].astype(F32)
    mean = jnp.mean(x, axis=-1, keepdims=True)
    xc = x - mean
    var = jnp.mean(xc * xc, axis=-1, keepdims=True)
    xn = xc / jnp.sqrt(var + 1e-5)
    xn = xn.astype(BF).astype(F32)
    r = jnp.sum(xn * wr_v[...].astype(F32).reshape(1, M), axis=-1, keepdims=True)
    gate_r = jax.nn.sigmoid(r)

    xn8 = jnp.concatenate([xn, xn], axis=0)
    xn8p = jnp.concatenate([xn8, jnp.zeros((8, 64), F32)], axis=1).astype(BF)
    xe = jnp.concatenate([_dot(xn8p[:, i * 128:(i + 1) * 128], exp2) for i in range(5)], axis=1)[:, :2 * M]
    lq = jnp.where(_iota((8, 2 * M), 1) % 2 == _iota((8, 2 * M), 0) // 4, xe, 0.0).astype(BF)

    cp(wq_v, wq_v, sems.at[2]).wait()
    for j in range(NP):
        cp(wuv32.at[:, j], wuv_v.at[j], sems.at[8]).start()
    cp(wuk_v, wuk_v, sems.at[3]).wait()

    def q_body(j, _):
        q = _dot(lq, pltpu.bitcast(wq_v[j], BF))
        z = _dot_nt(q.astype(BF), pltpu.bitcast(wuk_v[j], BF))
        z = jnp.where(_iota((8, 2 * DC), 1) % 2 == _iota((8, 2 * DC), 0) // 4, z * (D ** -0.5), 0.0)
        z_v[pl.ds(pl.multiple_of(j * 8, 8), 8), :] = z

    lax.fori_loop(0, NP, q_body, None)
    zb = z_v[...].astype(BF)
    for i in range(4):
        row_v[i] = _dot(zb[:, i * 256:(i + 1) * 256], cmp2)
    qs = [jnp.concatenate([row_v[i, pl.ds(b, H, stride=B), :] for i in range(4)], axis=1).astype(BF) for b in range(B)]

    nk = SK // KC
    for b in range(B):
        cp(ckv_hbm.at[b], ckv_v.at[b], sems.at[4 + b]).wait()

        def s_body(i, m):
            k0 = pl.multiple_of(i * KC, KC)
            s = _dot_nt(qs[b], ckv_v[b, pl.ds(k0, KC), :])
            s_v[i] = s
            for t in range(KC // 128):
                m = jnp.maximum(m, s[:, t * 128:(t + 1) * 128])
            return m

        m = lax.fori_loop(0, nk, s_body, jnp.full((H, 128), -jnp.inf, F32))
        m = jnp.max(m, axis=-1, keepdims=True)

        def pv_body(i, c):
            l, acc = c
            k0 = pl.multiple_of(i * KC, KC)
            p = jnp.exp(s_v[i] - m)
            for t in range(KC // 128):
                l = l + p[:, t * 128:(t + 1) * 128]
            return l, acc + _dot(p.astype(BF), ckv_v[b, pl.ds(k0, KC), :])

        l, acc = lax.fori_loop(0, nk, pv_body, (jnp.zeros((H, 128), F32), jnp.zeros((H, DC), F32)))
        acc = acc / jnp.sum(l, axis=-1, keepdims=True)
        for i in range(4):
            row_v[i, pl.ds(b, H, stride=B), :] = acc[:, i * 128:(i + 1) * 128]

    for i in range(4):
        e = _dot(row_v[i].astype(BF), exp2)
        z_v[:, i * 256:(i + 1) * 256] = jnp.where(
            _iota((128, 256), 1) % 2 == (_iota((128, 256), 0) // 4) % 2, e, 0.0)
    cp(wuv_v, wuv_v, sems.at[8]).wait()
    cp(wo_hbm, wo_v, sems.at[9]).wait()

    def o_body(j, acc):
        lv = z_v[pl.ds(pl.multiple_of(j * 8, 8), 8), :].astype(BF)
        ctx = _dot(lv, pltpu.bitcast(wuv_v[j], BF))
        return acc + _dot_nt(ctx.astype(BF), wo_v[j])

    so = lax.fori_loop(0, NP, o_body, jnp.zeros((8, 2 * M), F32))
    s_att = so[0:4, 0:M] + so[4:8, M:2 * M]

    z4 = jnp.zeros((4, M), F32)
    lf = jnp.concatenate([jnp.concatenate([xn, z4], axis=1), jnp.concatenate([z4, xn], axis=1)], axis=0).astype(BF)
    cp(wgu_v, wgu_v, sems.at[10]).wait()
    for i in range(F // FC):
        gu = _dot(lf, wgu_v[:, i * FC:(i + 1) * FC])
        h_v[:, i * FC:(i + 1) * FC] = jax.nn.silu(gu[0:4]) * gu[4:8]
    hh = jnp.concatenate([h_v[:, 0:F // 2], h_v[:, F // 2:F]], axis=0).astype(BF)
    cp(wd_v, wd_v, sems.at[11]).wait()
    yo = jnp.zeros((8, 2 * M), F32)
    for i in range(F // 2 // DCc):
        yo = yo + _dot_nt(hh[:, i * DCc:(i + 1) * DCc], wd_v[:, i * DCc:(i + 1) * DCc])
    y = (yo[0:4, 0:M] + yo[4:8, M:2 * M]) * gate_r
    g = jax.nn.silu(xn + (xn * 0.0 + y))
    o_ref[...] = (x + s_att * g).astype(o_ref.dtype)


@jax.jit
def pallas_recurrent_scan__compressed_kv_cla__moe_arch_mod__decode_kernel(
        A_x, A_c_kv, A_w_q, A_w_uk, A_w_uv, A_w_o, B_x, B_w_r, B_w_gate, B_w_up, B_w_down):
    del B_x
    hbm = pl.BlockSpec(memory_space=pltpu.HBM)
    wo_t = jnp.transpose(A_w_o, (0, 2, 1)).reshape(NP, 2 * M, D)
    out = pl.pallas_call(
        _kernel,
        out_shape=jax.ShapeDtypeStruct((B, M), A_x.dtype),
        in_specs=[hbm] * 10,
        scratch_shapes=[
            pltpu.VMEM((B, M), BF),
            pltpu.VMEM((M,), BF),
            pltpu.VMEM((B, SK, DC), BF),
            pltpu.VMEM((NP, M, D), jnp.uint32),
            pltpu.VMEM((NP, DC, D), jnp.uint32),
            pltpu.VMEM((NP, DC, D), jnp.uint32),
            pltpu.VMEM((NP, 2 * M, D), BF),
            pltpu.VMEM((2 * M, F), BF),
            pltpu.VMEM((2 * M, F // 2), BF),
            pltpu.VMEM((B * H, 2 * DC), F32),
            pltpu.VMEM((4, B * H, 128), F32),
            pltpu.VMEM((SK // KC, H, KC), F32),
            pltpu.VMEM((SK // KC, H, KC), BF),
            pltpu.VMEM((B, F), F32),
            pltpu.SemaphoreType.DMA((12,)),
        ],
        compiler_params=pltpu.CompilerParams(vmem_limit_bytes=100 * 1024 * 1024),
    )(A_x.reshape(B, M), B_w_r, A_c_kv, A_w_q, A_w_uk, A_w_uv, wo_t, B_w_gate, B_w_up, B_w_down.T)
    return out.reshape(B, 1, M)
```

```python
import functools
import jax
import jax.numpy as jnp
import numpy as np
from jax import lax
from jax.experimental import pallas as pl
from jax.experimental.pallas import tpu as pltpu

B, M, H, D, DC, SK, F = 4, 576, 32, 128, 512, 4096, 4608
NP = H // 2
BF = jnp.bfloat16
F32 = jnp.float32
NT = (((1,), (1,)), ((), ()))
ds = pl.ds


def _dot(a, b):
    return jnp.dot(a, b, preferred_element_type=F32)


def _dot_nt(a, b):
    return lax.dot_general(a, b, NT, preferred_element_type=F32)


def _iota(shape, dim):
    return lax.broadcasted_iota(jnp.int32, shape, dim)


def _mult(x, n):
    return x if isinstance(x, int) else pl.multiple_of(x, n)


def _onehot(cond):
    return cond.astype(F32).astype(BF)


def _kernel(x_hbm, wr_hbm, ckv_hbm, wq_hbm, wuk_hbm, wuv_hbm, wo_hbm, wg_hbm, wu_hbm, wd_hbm,
            o_ref,
            x_v, wr_v, ckv_v, wq_v, wuk_v, wuv_v, wo_v, wg_v, wu_v, wd_v,
            xn_v, lhs_v, q_v, z_v, row_v, qb_v, s_v, m_v, ctx_v, h_v, so_v, sems, xsem,
            *, gap, gap2, compute, dma, scopes, L):
    def group(*members):
        def copies(j):
            bulk, singles, whole = [], [], []
            left = sum(m[4] for m in members) - 2
            for src, dst, n, lo, cnt in members:
                r = ds(_mult(j * n, n), n)
                k = min(cnt, left)
                left -= k
                if k:
                    bulk.append((src.at[ds(lo, k), r], dst.at[ds(lo, k), r]))
                singles += [(src.at[lo + t, r], dst.at[lo + t, r]) for t in range(k, cnt)]
                whole.append((src.at[ds(lo, cnt), r], dst.at[ds(lo, cnt), r]))
            return bulk, singles, whole
        return copies

    wq32, wuk32, wuv32 = (r.bitcast(jnp.uint32) for r in (wq_hbm, wuk_hbm, wuv_hbm))
    phases = [
        (32, group((wq32, wq_v, 32, 0, 9))),
        (32, group((wuk32, wuk_v, 32, 0, 8), (ckv_hbm, ckv_v, 16, 0, 4))),
        (32, group((ckv_hbm, ckv_v, 16, 4, 12))),
        (32, group((ckv_hbm, ckv_v, 16, 16, 12))),
        (32, group((wuv32, wuv_v, 32, 0, 8), (ckv_hbm, ckv_v, 16, 28, 4))),
        (36, group((wg_hbm, wg_v, 64, 0, 9))),
        (36, group((wu_hbm, wu_v, 64, 0, 9))),
        (36, group((wd_hbm, wd_v, 64, 0, 9))),
        (32, group((wo_hbm, wo_v, 64, 0, 9))),
    ]

    def slot(p, j):
        return (sum(n for n, _ in phases[:p]) % L + j) % L

    def arrive(p, j):
        for c in phases[p][1](j)[2]:
            pltpu.make_async_copy(*c, sems.at[slot(p, j)]).wait()

    def issue(p, j, t):
        bulk, singles, _ = phases[p][1](j)
        sem = sems.at[slot(p, j)]
        pltpu.make_async_copy(*singles[t], sem).start()
        if t == 0:
            for c in bulk:
                pltpu.make_async_copy(*c, sem).start(priority=1)

    def issue_ahead(p, j, t, j_min, j_max):
        n = phases[p][0]
        more = p + 1 < len(phases)
        if j_max + L < n:
            issue(p, j + L, t)
        elif j_min + L >= n:
            if more:
                issue(p + 1, j + L - n, t)
        else:
            pl.when(j + L < n)(lambda: issue(p, j + L, t))
            if more:
                pl.when(j + L >= n)(lambda: issue(p + 1, j + L - n, t))

    def run(p, first, count, k, work=None, carry=None, shift=0, shift_max=0):
        work = work if compute else None
        halves = [(s, t) for s in range(k) for t in range(2)]
        done = p + 1 == len(phases) and first + L >= phases[p][0]

        def issue_some(j, todo):
            for n, (s, t) in enumerate(todo):
                if n:
                    pl.delay(gap2)
                issue_ahead(p, j + s, t, first + s, first + s + shift_max + (count - 1) * k)

        def body(i, c):
            j = first + shift + i * k
            if not dma:
                return c if work is None else work(i, c)
            for s in range(k):
                arrive(p, j + s)
            if done:
                return c if work is None else work(i, c)
            issue_some(j, halves[:k])
            if work is None:
                pl.delay(gap)
            else:
                pl.delay(1)
                c = work(i, c)
                pl.delay(1)
            issue_some(j, halves[k:])
            return c
        if scopes:
            with jax.named_scope(f"ph{p}_{first}"):
                return lax.fori_loop(0, count, body, carry)
        return lax.fori_loop(0, count, body, carry)

    cx = pltpu.make_async_copy(x_hbm, x_v, xsem.at[0])
    cr = pltpu.make_async_copy(wr_hbm, wr_v, xsem.at[1])
    if dma:
        for j in range(L):
            for c in phases[0][1](j)[2]:
                pltpu.make_async_copy(*c, sems.at[slot(0, j)]).start(priority=1)
    cx.start()
    cr.start()

    run(0, 0, 2, 1)
    cx.wait()
    cr.wait()
    x = x_v[...].astype(F32)
    xc = x - jnp.mean(x, axis=-1, keepdims=True)
    var = jnp.mean(xc * xc, axis=-1, keepdims=True)
    xn = (xc / jnp.sqrt(var + 1e-5)).astype(BF).astype(F32)
    xn_v[...] = xn

    def spread(group):
        n = _iota((128, 256), 1)
        e = _onehot(_iota((128, 256), 0) == n // (2 * group) * group + n % group)
        xn = xn_v[...]
        xn = jnp.concatenate([xn, xn], axis=0)
        xn = jnp.concatenate([xn, jnp.zeros((8, 64), F32)], axis=1).astype(BF)
        xe = jnp.concatenate([_dot(xn[:, i * 128:(i + 1) * 128], e) for i in range(5)], axis=1)[:, :2 * M]
        lhs_v[...] = jnp.where(_iota((8, 2 * M), 1) // group % 2 == _iota((8, 2 * M), 0) // 4, xe, 0.0)

    spread(1)
    run(0, 2, 30, 1)

    def pair_rows(ref, j):
        w = [ref[r, ds(j, ref.shape[1] // NP, stride=NP), :] for r in range(ref.shape[0])]
        return pltpu.bitcast(jnp.concatenate(w, axis=0), BF)

    def q_proj(j, c):
        q_v[j] = _dot(lhs_v[...].astype(BF), pair_rows(wq_v, j))
        return c

    run(1, 0, NP, 2, q_proj)

    def absorb(j, c):
        z = _dot_nt(q_v[j].astype(BF), pair_rows(wuk_v, j))
        keep = _iota((8, 2 * DC), 1) % 2 == _iota((8, 2 * DC), 0) // 4
        z_v[ds(_mult(j * 8, 8), 8), :] = jnp.where(keep, z * (D ** -0.5), 0.0)
        return c

    run(2, 0, NP, 2, absorb)
    if compute:
        cmp2 = _onehot(_iota((256, 128), 0) // 2 == _iota((256, 128), 1))
        for i in range(4):
            row_v[i] = _dot(z_v[:, i * 256:(i + 1) * 256].astype(BF), cmp2)
        for b in range(B):
            qb_v[b] = jnp.concatenate([row_v[i, ds(b, H, stride=B), :] for i in range(4)], axis=1).astype(BF)

    def scores(r, mx, half=None):
        if half is None:
            s = _dot_nt(qb_v[r // 8], ckv_v[r])
            s_v[r, 0] = s[:, :256]
            s_v[r, 1] = s[:, 256:]
        else:
            s = _dot_nt(qb_v[r // 8], ckv_v[r, ds(_mult(half * 256, 256), 256), :])
            s_v[r, half] = s
        for t in range(s.shape[1] // 128):
            mx = jnp.maximum(mx, s[:, t * 128:(t + 1) * 128])
        return mx

    def keep_max(b, mx):
        if compute:
            m_v[b] = jnp.broadcast_to(jnp.max(mx, axis=-1, keepdims=True), mx.shape)

    def values(r, c):
        l, acc = c
        m = m_v[r // 8]
        p = [jnp.exp(s_v[r, t // 2, :, (t % 2) * 128:(t % 2 + 1) * 128] - m) for t in range(4)]
        l = l + ((p[0] + p[1]) + (p[2] + p[3]))
        return l, acc + _dot(jnp.concatenate(p, axis=1).astype(BF), ckv_v[r])

    def keep_context(b, c):
        if compute:
            out = c[1] / jnp.sum(c[0], axis=-1, keepdims=True)
            for i in range(4):
                row_v[i, ds(b, H, stride=B), :] = out[:, i * 128:(i + 1) * 128]

    mx0 = jnp.full((H, 128), -jnp.inf, F32)
    pv0 = (jnp.zeros((H, 128), F32), jnp.zeros((H, DC), F32))

    def first_scores(b, _):
        keep_max(b, run(3, 0, 8, 2, lambda j, c: scores(8 * b + j, c), mx0, 16 * b, 16))

    lax.fori_loop(0, 2, first_scores, None)

    def first_values(b, mx):
        mx, pv = run(4, 0, 8, 2, lambda j, c: (scores(16 + 4 * b + j // 2, c[0], j % 2), values(8 * b + j, c[1])),
                     (mx, pv0), 16 * b, 16)
        keep_context(b, pv)
        return mx

    keep_max(2, lax.fori_loop(0, 2, first_values, mx0))
    mx, pv = run(5, 0, 8, 3, lambda j, c: (scores(24 + j, c[0]), values(16 + j, c[1])), (mx0, pv0))
    keep_context(2, pv)
    keep_max(3, mx)
    keep_context(3, run(5, 24, 4, 3, lambda j, c: values(25 + 2 * j, values(24 + 2 * j, c)), pv0))

    run(6, 0, 1, 1)
    if compute:
        exp2 = _onehot(_iota((128, 256), 0) == _iota((128, 256), 1) // 2)
        for i in range(4):
            e = _dot(row_v[i].astype(BF), exp2)
            keep = _iota((128, 256), 1) % 2 == (_iota((128, 256), 0) // 4) % 2
            z_v[:, i * 256:(i + 1) * 256] = jnp.where(keep, e, 0.0)
    run(6, 1, 2, 1)
    spread(8)
    so_v[...] = jnp.zeros(so_v.shape, F32)
    run(6, 3, 1, 1)

    def up_v(i, c):
        for j in (2 * i, 2 * i + 1):
            ctx_v[j] = _dot(z_v[ds(_mult(j * 8, 8), 8), :].astype(BF), pair_rows(wuv_v, j))
        return c

    run(6, 4, 8, 4, up_v)

    def tile_pair(ref, j, bands=range(8)):
        w = [ref[r, ds(_mult(band * 288 + j * 16, 16), 16), :] for r in range(9) for band in bands]
        return jnp.concatenate(w, axis=0)

    def gate_up(i, c):
        lhs = lhs_v[...].astype(BF)
        for j in (2 * i, 2 * i + 1):
            h_v[j] = jax.nn.silu(_dot(lhs, tile_pair(wg_v, j))) * _dot(lhs, tile_pair(wu_v, j))
        return c

    def down(js, bands, c):
        for j in js:
            c = c + _dot_nt(h_v[j].astype(BF), tile_pair(wd_v, j, bands))
        return c

    run(7, 0, 9, 2, gate_up)
    y0 = run(7, 18, 6, 3, lambda i, c: down((3 * i, 3 * i + 1, 3 * i + 2), range(4), c), jnp.zeros((8, M), F32))

    def out_proj(j, c=None):
        for r in range(9):
            tile = 16 * r + j
            w = wo_v[r, ds(_mult(j * 128, 128), 128), :]
            so_v[tile % 9] += _dot_nt(ctx_v[tile // 9].astype(BF), w)
        return c

    y1 = run(8, 0, 9, 2, lambda i, c: down((2 * i, 2 * i + 1), range(4, 8), out_proj(i, c)), jnp.zeros((8, M), F32))
    pad = jnp.zeros((8, 64), F32)
    yo = jnp.concatenate([y0, pad, y1, pad], axis=1)
    yo = jnp.where(_iota(yo.shape, 1) // 8 % 2 == _iota(yo.shape, 0) // 4, yo, 0.0)
    parts = []
    for _ in range(3):
        parts.append(yo.astype(BF).astype(F32))
        yo = yo - parts[-1]
    parts = jnp.concatenate(parts + [jnp.zeros_like(yo)], axis=0).astype(BF)
    n = _iota((256, 128), 0)
    cmp8 = _onehot(n // 64 % 2 * 64 + n // 128 * 32 + n // 16 % 4 * 8 + n % 8 == _iota((256, 128), 1))
    y = jnp.concatenate(
        [_dot(jnp.concatenate([parts[:, i * 128:(i + 1) * 128], parts[:, 640 + i * 128:768 + i * 128]], axis=1), cmp8)
         for i in range(5)], axis=1)
    y = y[0:8] + y[8:16] + y[16:24]
    y = (y[0:4] + y[4:8])[:, :M]
    xn = xn_v[...]
    r = jnp.sum(xn * wr_v[...].astype(F32).reshape(1, M), axis=-1, keepdims=True)
    g = jax.nn.silu(xn + (xn * 0.0 + y * jax.nn.sigmoid(r)))
    run(8, 18, (14 - L) // 2, 2, lambda i, c: out_proj(9 + i))
    run(8, 32 - L, L // 2, 2, lambda i, c: out_proj(16 - L // 2 + i))
    so = jnp.concatenate([so_v[i] for i in range(9)], axis=1)
    s_att = so[0:4, 0:M] + so[4:8, M:2 * M]
    o_ref[...] = (x_v[...].astype(F32) + s_att * g).astype(o_ref.dtype)


def _tiles(w):
    return w.reshape(72, 8, 36, 128).transpose(0, 2, 1, 3).reshape(9, 2304, 128)


def make(gap=60, gap2=30, compute=True, dma=True, scopes=False, L=12, **cp):
    @jax.jit
    def kernel_fn(A_x, A_c_kv, A_w_q, A_w_uk, A_w_uv, A_w_o, B_x, B_w_r, B_w_gate, B_w_up, B_w_down):
        del B_x
        hbm = pl.BlockSpec(memory_space=pltpu.HBM)
        params = dict(vmem_limit_bytes=100 * 1024 * 1024, disable_semaphore_checks=True, disable_bounds_checks=True)
        params.update(cp)
        out = pl.pallas_call(
            functools.partial(_kernel, gap=gap, gap2=gap2, compute=compute, dma=dma, scopes=scopes, L=L),
            out_shape=jax.ShapeDtypeStruct((B, M), A_x.dtype),
            in_specs=[hbm] * 10,
            scratch_shapes=[
                pltpu.VMEM((B, M), BF),
                pltpu.VMEM((M,), BF),
                pltpu.VMEM((32, 512, DC), BF),
                pltpu.VMEM((9, 1024, D), jnp.uint32),
                pltpu.VMEM((8, 1024, D), jnp.uint32),
                pltpu.VMEM((8, 1024, D), jnp.uint32),
                pltpu.VMEM((9, 2048, D), BF),
                pltpu.VMEM((9, 2304, 128), BF),
                pltpu.VMEM((9, 2304, 128), BF),
                pltpu.VMEM((9, 2304, 128), BF),
                pltpu.VMEM((B, M), F32),
                pltpu.VMEM((8, 2 * M), F32),
                pltpu.VMEM((NP, 8, D), F32),
                pltpu.VMEM((B * H, 2 * DC), F32),
                pltpu.VMEM((4, B * H, 128), F32),
                pltpu.VMEM((B, H, DC), BF),
                pltpu.VMEM((32, 2, H, 256), F32),
                pltpu.VMEM((B, H, 128), F32),
                pltpu.VMEM((NP, 8, D), F32),
                pltpu.VMEM((18, 8, 128), F32),
                pltpu.VMEM((9, 8, 128), F32),
                pltpu.SemaphoreType.DMA((L,)),
                pltpu.SemaphoreType.DMA((2,)),
            ],
            compiler_params=pltpu.CompilerParams(**params),
        )(A_x.reshape(B, M), B_w_r, A_c_kv.reshape(32, 512, DC), A_w_q.reshape(9, 2048, D),
          A_w_uk.reshape(8, 2048, D), A_w_uv.reshape(8, 2048, D),
          jnp.transpose(A_w_o, (0, 2, 1)).reshape(9, 2048, D),
          _tiles(B_w_gate), _tiles(B_w_up), _tiles(B_w_down.T))
        return out.reshape(B, 1, M)
    return kernel_fn


pallas_recurrent_scan__compressed_kv_cla__moe_arch_mod__decode_kernel = make()
```

```python
import contextlib
import functools

import jax
import jax.numpy as jnp
from jax import lax
from jax.experimental import pallas as pl
from jax.experimental.pallas import tpu as pltpu

B, M, H, D, DC, SK, F = 4, 576, 32, 128, 512, 4096, 4608
NP = H // 2
AHEAD = 6
RING = 8
BF = jnp.bfloat16
F32 = jnp.float32
ds = pl.ds


def _dot(a, b):
    return jnp.dot(a, b, preferred_element_type=F32)


def _dot_nt(a, b):
    return lax.dot_general(a, b, (((1,), (1,)), ((), ())), preferred_element_type=F32)


def _iota(shape, dim):
    return lax.broadcasted_iota(jnp.int32, shape, dim)


def _mult(x, n):
    return x if isinstance(x, int) else pl.multiple_of(x, n)


def _onehot(cond):
    return cond.astype(F32).astype(BF)


def _kernel(x_hbm, wr_hbm, ckv_hbm, wq_hbm, wuk_hbm, wuv_hbm, wo_hbm, wg_hbm, wu_hbm, wd_hbm,
            o_ref,
            x_v, wr_v, ckv_v, wq_v, wuk_v, wuv_v, wo_v, wg_v, wu_v, wd_v,
            xn_v, lhs_v, q_v, z_v, row_v, qb_v, s_v, m_v, ctx_v, h_v, so_v, fin_v, pad_v, sems, xsem,
            *, long, short, n9, scopes, compute):
    scope = jax.named_scope if scopes else (lambda n: contextlib.nullcontext())

    def part(src, dst, rows, regions, first, count=1):
        r = ds(_mult(first * rows, rows), rows * count)
        return src.at[regions, r], dst.at[regions, r]

    def nine_regions(src, dst, rows, singles):
        p = functools.partial(part, src, dst, rows)
        if singles == 4:
            return lambda j: ([p(ds(0, 7), 2 * j), p(ds(0, 7), 2 * j + 1)],
                              [p(7, 2 * j), p(8, 2 * j), p(7, 2 * j + 1), p(8, 2 * j + 1)])
        return lambda j: ([p(ds(0, 7), 2 * j), p(ds(0, 8), 2 * j + 1)],
                          [p(7, 2 * j), p(8, 2 * j), p(8, 2 * j + 1)])

    def twelve_regions(first, weight=None):
        cache = functools.partial(part, ckv_hbm, ckv_v, 16)
        count = 4 if weight else 12

        def copies(j):
            bulk = []
            for piece in (2 * j, 2 * j + 1):
                if weight:
                    bulk.append(part(*weight, 32, ds(0, 8), piece))
                bulk.append(cache(ds(first, count - 2), piece))
            return bulk, [cache(first + count - 2 + t, piece) for piece in (2 * j, 2 * j + 1) for t in range(2)]
        return copies

    def wo_regions(j):
        p = functools.partial(part, wo_hbm, wo_v, 64)
        return ([p(ds(0, 7), 2 * j), p(ds(0, 7), 2 * j + 1)],
                [p(7, 2 * j), p(8, 2 * j + 2), p(7, 2 * j + 1), p(8, 2 * j + 3)])

    wq32, wuk32, wuv32 = (r.bitcast(jnp.uint32) for r in (wq_hbm, wuk_hbm, wuv_hbm))
    phases = [
        (16, nine_regions(wq32, wq_v, 32, n9[0])),
        (16, twelve_regions(0, (wuk32, wuk_v))),
        (16, twelve_regions(4)),
        (16, twelve_regions(16)),
        (16, twelve_regions(28, (wuv32, wuv_v))),
        (18, nine_regions(wg_hbm, wg_v, 64, n9[1])),
        (18, nine_regions(wu_hbm, wu_v, 64, n9[2])),
        (18, nine_regions(wd_hbm, wd_v, 64, n9[3])),
        (15, wo_regions),
    ]

    def copy(p, j, refs):
        return pltpu.make_async_copy(*refs, sems.at[(sum(n for n, _ in phases[:p]) + j) & (RING - 1)])

    def pause(n):
        def tick(_, c):
            v = pad_v[...]
            pad_v[...] = v * v
            return c
        lax.fori_loop(0, n, tick, 0)

    def wait(p, j, k):
        bulk, singles = phases[p][1](j)
        half = len(bulk) // 2
        with (jax.named_scope(f"w{p}") if scopes == 2 and k == 1 else contextlib.nullcontext()):
            for refs in (bulk[:half], bulk[half:], singles)[k]:
                copy(p, j, refs).wait()

    def start(p, j, early):
        bulk, singles = phases[p][1](j)
        if early:
            for refs in bulk:
                copy(p, j, refs).start(priority=1)
            pause(short)
        for t, refs in enumerate(singles[:2] if early else singles[2:]):
            if t:
                pause(long)
            copy(p, j, refs).start()

    def start_ahead(p, j, early, j_min, j_max):
        n = phases[p][0]
        if j_max + AHEAD < n:
            start(p, j + AHEAD, early)
        elif j_min + AHEAD >= n:
            start(p + 1, j + AHEAD - n, early)
        else:
            pl.when(j + AHEAD < n)(lambda: start(p, j + AHEAD, early))
            pl.when(j + AHEAD >= n)(lambda: start(p + 1, j + AHEAD - n, early))

    def run(p, first, count, work=None, carry=None, shift=0, shift_max=0):
        def body(i, c):
            j = first + shift + i
            span = (first, first + shift_max + count - 1)
            wait(p, j, 0)
            start_ahead(p, j, True, *span)
            wait(p, j, 1)
            if work is not None and compute:
                c = work(i, c)
            wait(p, j, 2)
            start_ahead(p, j, False, *span)
            return c
        with scope(f"ph{p}_{first}"):
            return lax.fori_loop(0, count, body, carry)

    x_copy = pltpu.make_async_copy(x_hbm, x_v, xsem.at[0])
    wr_copy = pltpu.make_async_copy(wr_hbm, wr_v, xsem.at[1])
    for j in range(AHEAD):
        for refs in phases[0][1](j)[0]:
            copy(0, j, refs).start(priority=1)
    x_copy.start()
    wr_copy.start()
    pad_v[...] = jnp.zeros(pad_v.shape, F32)
    for j in range(AHEAD):
        for refs in phases[0][1](j)[1]:
            pause(long)
            copy(0, j, refs).start()

    run(0, 0, 1)
    x_copy.wait()
    wr_copy.wait()
    x = x_v[...].astype(F32)
    xc = x - jnp.mean(x, axis=-1, keepdims=True)
    var = jnp.mean(xc * xc, axis=-1, keepdims=True)
    xn_v[...] = (xc / jnp.sqrt(var + 1e-5)).astype(BF).astype(F32)

    def spread(group):
        n = _iota((128, 256), 1)
        e = _onehot(_iota((128, 256), 0) == n // (2 * group) * group + n % group)
        xn = xn_v[...]
        xn = jnp.concatenate([xn, xn], axis=0)
        xn = jnp.concatenate([xn, jnp.zeros((8, 64), F32)], axis=1).astype(BF)
        xe = jnp.concatenate([_dot(xn[:, i * 128:(i + 1) * 128], e) for i in range(5)], axis=1)[:, :2 * M]
        lhs_v[...] = jnp.where(_iota((8, 2 * M), 1) // group % 2 == _iota((8, 2 * M), 0) // 4, xe, 0.0)

    spread(1)
    run(0, 1, 15)

    def pair_rows(ref, j):
        w = [ref[r, ds(j, ref.shape[1] // NP, stride=NP), :] for r in range(ref.shape[0])]
        return pltpu.bitcast(jnp.concatenate(w, axis=0), BF)

    def q_proj(j, c):
        q_v[j] = _dot(lhs_v[...].astype(BF), pair_rows(wq_v, j))
        return c

    run(1, 0, NP, q_proj)

    def absorb(j, c):
        z = _dot_nt(q_v[j].astype(BF), pair_rows(wuk_v, j))
        keep = _iota((8, 2 * DC), 1) % 2 == _iota((8, 2 * DC), 0) // 4
        z_v[ds(_mult(j * 8, 8), 8), :] = jnp.where(keep, z * (D ** -0.5), 0.0)
        return c

    run(2, 0, NP, absorb)
    if compute:
        drop_e = _onehot(_iota((256, 128), 0) // 2 == _iota((256, 128), 1))
        for i in range(4):
            row_v[i] = _dot(z_v[:, i * 256:(i + 1) * 256].astype(BF), drop_e)
        for b in range(B):
            qb_v[b] = jnp.concatenate([row_v[i, ds(b, H, stride=B), :] for i in range(4)], axis=1).astype(BF)

    def scores(r, mx, half=None):
        if half is None:
            s = _dot_nt(qb_v[r >> 3], ckv_v[r])
            s_v[r, 0] = s[:, :256]
            s_v[r, 1] = s[:, 256:]
        else:
            s = _dot_nt(qb_v[r >> 3], ckv_v[r, ds(_mult(half * 256, 256), 256), :])
            s_v[r, half] = s
        for t in range(s.shape[1] // 128):
            mx = jnp.maximum(mx, s[:, t * 128:(t + 1) * 128])
        return mx

    def keep_max(b, mx):
        m_v[b] = jnp.broadcast_to(jnp.max(mx, axis=-1, keepdims=True), mx.shape)

    def values(r, c):
        l, acc = c
        m = m_v[r >> 3]
        p = [jnp.exp(s_v[r, t // 2, :, (t % 2) * 128:(t % 2 + 1) * 128] - m) for t in range(4)]
        l = l + ((p[0] + p[1]) + (p[2] + p[3]))
        return l, acc + _dot(jnp.concatenate(p, axis=1).astype(BF), ckv_v[r])

    def keep_context(b, c):
        out = c[1] / jnp.sum(c[0], axis=-1, keepdims=True)
        for i in range(4):
            row_v[i, ds(b, H, stride=B), :] = out[:, i * 128:(i + 1) * 128]

    mx0 = jnp.full((H, 128), -jnp.inf, F32)
    pv0 = (jnp.zeros((H, 128), F32), jnp.zeros((H, DC), F32))

    def first_scores(b, _):
        keep_max(b, run(3, 0, 8, lambda j, c: scores(8 * b + j, c), mx0, 8 * b, 8))

    lax.fori_loop(0, 2, first_scores, None)

    def first_values(b, mx):
        mx, pv = run(4, 0, 8, lambda j, c: (scores(16 + 4 * b + (j >> 1), c[0], j & 1), values(8 * b + j, c[1])),
                     (mx, pv0), 8 * b, 8)
        keep_context(b, pv)
        return mx

    keep_max(2, lax.fori_loop(0, 2, first_values, mx0))
    mx, pv = run(5, 0, 8, lambda j, c: (scores(24 + j, c[0]), values(16 + j, c[1])), (mx0, pv0))
    keep_context(2, pv)
    keep_max(3, mx)
    keep_context(3, run(5, 8, 8, lambda j, c: values(24 + j, c), pv0))
    run(5, 16, 1)
    add_e = _onehot(_iota((128, 256), 0) == _iota((128, 256), 1) // 2)
    keep = _iota((128, 256), 1) % 2 == (_iota((128, 256), 0) // 4) % 2
    for i in range(4):
        z_v[:, i * 256:(i + 1) * 256] = jnp.where(keep, _dot(row_v[i].astype(BF), add_e), 0.0)
    run(5, 17, 1)

    def up_v(j, c):
        ctx_v[j] = _dot(z_v[ds(_mult(j * 8, 8), 8), :].astype(BF), pair_rows(wuv_v, j))
        return c

    run(6, 0, NP, up_v)
    spread(8)
    so_v[...] = jnp.zeros(so_v.shape, F32)
    run(6, 16, 2)

    def tile_pair(ref, j, bands=range(8)):
        w = [ref[r, ds(_mult(band * 288 + j * 16, 16), 16), :] for r in range(9) for band in bands]
        return jnp.concatenate(w, axis=0)

    def gate_up(i, c):
        lhs = lhs_v[...].astype(BF)
        for j in (2 * i, 2 * i + 1):
            h_v[j] = jax.nn.silu(_dot(lhs, tile_pair(wg_v, j))) * _dot(lhs, tile_pair(wu_v, j))
        return c

    def down(js, bands, c):
        for j in js:
            c = c + _dot_nt(h_v[j].astype(BF), tile_pair(wd_v, j, bands))
        return c

    def out_proj(tiles):
        for r, j in tiles:
            tile = 16 * r + j
            pair = (tile * 57) >> 9
            so_v[tile - 9 * pair] += _dot_nt(ctx_v[pair].astype(BF), wo_v[r, ds(_mult(j * 128, 128), 128), :])

    first_tile = pltpu.make_async_copy(*part(wo_hbm, wo_v, 128, 8, 0), xsem.at[0])
    last_tiles = pltpu.make_async_copy(*part(wo_hbm, wo_v, 128, ds(0, 8), 15), xsem.at[1])
    first_tile.start(priority=1)
    run(7, 0, 9, gate_up)
    y0 = run(7, 9, 6, lambda i, c: down([3 * i + t for t in range(3)], range(4), c), jnp.zeros((8, M), F32))
    y1 = run(7, 15, 3, lambda i, c: down([6 * i + t for t in range(6)], (4, 5), c), jnp.zeros((8, M // 2), F32))
    first_tile.wait()
    out_proj([(8, 0)])

    last = len(phases) - 1
    late = 4 * (phases[last][0] - AHEAD)

    def last_rounds(first, count, work=None, carry=None):
        def body(i, c):
            def ahead():
                if first + AHEAD < phases[last][0]:
                    for refs in wo_regions(i + AHEAD)[0]:
                        copy(last, i + AHEAD, refs).start(priority=1)
                for k in range(3):
                    if k:
                        pause(long)
                    j, t = AHEAD + ((3 * i + k) >> 2), (3 * i + k) & 3
                    copy(last, j, part(wo_hbm, wo_v, 64, 7 + (t & 1), 2 * j + (t >> 1) + 2 * (t & 1))).start()

            wait(last, i, 0)
            ahead() if 3 * (first + count) <= late else pl.when(3 * i < late)(ahead)
            wait(last, i, 1)
            wait(last, i, 2)
            if compute:
                out_proj([(8, i + 1)] + [(r, i) for r in range(8)])
                c = c if work is None else work(i, c)
            return c
        with scope(f"last_{first}"):
            return lax.fori_loop(first, first + count, body, carry)

    y2 = last_rounds(0, 9, lambda i, c: down((2 * i, 2 * i + 1), (6, 7), c), jnp.zeros((8, M // 2), F32))
    last_tiles.start(priority=1)
    y0, y1, y2 = (jnp.concatenate([v, jnp.zeros((8, v.shape[1] // 9), F32)], axis=1) for v in (y0, y1, y2))
    yo = jnp.concatenate([v[:, i * n:(i + 1) * n] for i in range(5) for v, n in ((y0, 128), (y1, 64), (y2, 64))], axis=1)
    yo = jnp.where(_iota(yo.shape, 1) // 8 % 2 == _iota(yo.shape, 0) // 4, yo, 0.0)
    parts = []
    for _ in range(3):
        parts.append(yo.astype(BF).astype(F32))
        yo = yo - parts[-1]
    parts = jnp.concatenate(parts + [jnp.zeros_like(yo)], axis=0).astype(BF)
    n = _iota((256, 128), 0)
    region = jnp.where(n < 128, n // 64, n // 32 % 2)
    band = jnp.where(n < 128, n // 16 % 4, n // 64 * 2 + n // 16 % 2)
    in_order = _onehot(region * 64 + band * 8 + n % 8 == _iota((256, 128), 1))
    y = jnp.concatenate([_dot(parts[:, i * 256:(i + 1) * 256], in_order) for i in range(5)], axis=1)
    y = y[0:8] + y[8:16] + y[16:24]
    y = (y[0:4] + y[4:8])[:, :M]
    xn = xn_v[...]
    r = jnp.sum(xn * wr_v[...].astype(F32).reshape(1, M), axis=-1, keepdims=True)
    fin_v[...] = jnp.zeros(fin_v.shape, F32)
    fin_v[0, 0:4, 0:M] = jax.nn.silu(xn + (xn * 0.0 + y * jax.nn.sigmoid(r)))
    fin_v[1, 0:4, 0:M] = x_v[...].astype(F32)
    last_rounds(9, 6)

    with scope("final"):
        last_tiles.wait()
        low = _iota((8, 128), 1) < 64
        odd = [pltpu.roll(pltpu.roll(so_v[4 + t], 4, 0), 64, 1) for t in range(5)]
        s = [so_v[t] + jnp.where(low, odd[t], odd[min(t + 1, 4)]) for t in range(5)]
        for r in (1, 4, 5, 0, 2, 3, 6, 7):
            head, col = divmod(2048 * r + 1920, M)
            lhs = ctx_v[head // 2]
            lhs = pltpu.roll(lhs, 4, 0) if head % 2 else lhs
            z = _dot_nt(lhs.astype(BF), wo_v[r, ds(1920, 128), :])
            if col == 512:
                s[4] += jnp.where(low, z, 0.0)
                s[0] += jnp.where(low, pltpu.roll(pltpu.roll(z, 4, 0), 64, 1), 0.0)
            elif col % 128 == 0:
                s[col // 128] += z
            else:
                z = pltpu.roll(z, 64, 1)
                s[col // 128] += jnp.where(low, 0.0, z)
                s[col // 128 + 1] += jnp.where(low, z, 0.0)
        for t in range(5):
            lanes = slice(128 * t, 128 * (t + 1))
            out = fin_v[1, :, lanes] + s[t] * fin_v[0, :, lanes]
            n = min(128, M - 128 * t)
            o_ref[:, 128 * t:128 * t + n] = out[0:4, 0:n].astype(o_ref.dtype)


def _tiles(w):
    return w.reshape(72, 8, 36, 128).transpose(0, 2, 1, 3).reshape(9, 2304, 128)


def make(long=4, short=2, n9=(4, 3, 4, 3), scopes=False, compute=True, **cp):
    @jax.jit
    def kernel_fn(A_x, A_c_kv, A_w_q, A_w_uk, A_w_uv, A_w_o, B_x, B_w_r, B_w_gate, B_w_up, B_w_down):
        del B_x
        params = dict(vmem_limit_bytes=100 * 1024 * 1024, disable_semaphore_checks=True, disable_bounds_checks=True)
        params.update(cp)
        out = pl.pallas_call(
            functools.partial(_kernel, long=long, short=short, n9=n9, scopes=scopes, compute=compute),
            out_shape=jax.ShapeDtypeStruct((B, M), A_x.dtype),
            in_specs=[pl.BlockSpec(memory_space=pltpu.HBM)] * 10,
            scratch_shapes=[
                pltpu.VMEM((B, M), BF),
                pltpu.VMEM((M,), BF),
                pltpu.VMEM((32, 512, DC), BF),
                pltpu.VMEM((9, 1024, D), jnp.uint32),
                pltpu.VMEM((8, 1024, D), jnp.uint32),
                pltpu.VMEM((8, 1024, D), jnp.uint32),
                pltpu.VMEM((9, 2048, D), BF),
                pltpu.VMEM((9, 2304, 128), BF),
                pltpu.VMEM((9, 2304, 128), BF),
                pltpu.VMEM((9, 2304, 128), BF),
                pltpu.VMEM((B, M), F32),
                pltpu.VMEM((8, 2 * M), F32),
                pltpu.VMEM((NP, 8, D), F32),
                pltpu.VMEM((B * H, 2 * DC), F32),
                pltpu.VMEM((4, B * H, 128), F32),
                pltpu.VMEM((B, H, DC), BF),
                pltpu.VMEM((32, 2, H, 256), F32),
                pltpu.VMEM((B, H, 128), F32),
                pltpu.VMEM((NP, 8, D), F32),
                pltpu.VMEM((F // 256, 8, 128), F32),
                pltpu.VMEM((9, 8, 128), F32),
                pltpu.VMEM((2, 8, 640), F32),
                pltpu.VMEM((8, 128), F32),
                pltpu.SemaphoreType.DMA((RING,)),
                pltpu.SemaphoreType.DMA((2,)),
            ],
            compiler_params=pltpu.CompilerParams(**params),
        )(A_x.reshape(B, M), B_w_r, A_c_kv.reshape(32, 512, DC), A_w_q.reshape(9, 2048, D),
          A_w_uk.reshape(8, 2048, D), A_w_uv.reshape(8, 2048, D),
          jnp.transpose(A_w_o, (0, 2, 1)).reshape(9, 2048, D),
          _tiles(B_w_gate), _tiles(B_w_up), _tiles(B_w_down.T))
        return out.reshape(B, 1, M)
    return kernel_fn


pallas_recurrent_scan__compressed_kv_cla__moe_arch_mod__decode_kernel = make()
```

```python
import functools

import jax
import jax.numpy as jnp
from jax import lax
from jax.experimental import pallas as pl
from jax.experimental.pallas import tpu as pltpu

B, M, H, D, DC, F = 4, 576, 32, 128, 512, 4608
NP = H // 2
AHEAD = 6
RING = 8
LONG, SHORT = 4, 2
BF = jnp.bfloat16
F32 = jnp.float32
ds = pl.ds


def _dot(a, b):
    return jnp.dot(a, b, preferred_element_type=F32)


def _dot_nt(a, b):
    return lax.dot_general(a, b, (((1,), (1,)), ((), ())), preferred_element_type=F32)


def _iota(shape, dim):
    return lax.broadcasted_iota(jnp.int32, shape, dim)


def _mult(x, n):
    return x if isinstance(x, int) else pl.multiple_of(x, n)


def _onehot(cond):
    return cond.astype(F32).astype(BF)


def _kernel(x_hbm, wr_hbm, ckv_hbm, wq_hbm, wuk_hbm, wuv_hbm, wo_hbm, wg_hbm, wu_hbm, wd_hbm,
            o_ref,
            x_v, wr_v, ckv_v, wq_v, wuk_v, wuv_v, wo_v, wg_v, wu_v, wd_v,
            xn_v, lhs_v, q_v, z_v, row_v, qb_v, s_v, m_v, ctx_v, h_v, so_v, fin_v, pad_v, sems, xsem):
    def part(src, dst, rows, regions, first, count=1):
        r = ds(_mult(first * rows, rows), rows * count)
        return src.at[regions, r], dst.at[regions, r]

    def nine_regions(src, dst, rows, singles):
        p = functools.partial(part, src, dst, rows)
        if singles == 4:
            return lambda j: ([p(ds(0, 7), 2 * j), p(ds(0, 7), 2 * j + 1)],
                              [p(7, 2 * j), p(8, 2 * j), p(7, 2 * j + 1), p(8, 2 * j + 1)])
        return lambda j: ([p(ds(0, 7), 2 * j), p(ds(0, 8), 2 * j + 1)],
                          [p(7, 2 * j), p(8, 2 * j), p(8, 2 * j + 1)])

    def twelve_regions(first, weight=None):
        cache = functools.partial(part, ckv_hbm, ckv_v, 16)
        count = 4 if weight else 12

        def copies(j):
            bulk = []
            for piece in (2 * j, 2 * j + 1):
                if weight:
                    bulk.append(part(*weight, 32, ds(0, 8), piece))
                bulk.append(cache(ds(first, count - 2), piece))
            return bulk, [cache(first + count - 2 + t, piece) for piece in (2 * j, 2 * j + 1) for t in range(2)]
        return copies

    def wo_regions(j):
        p = functools.partial(part, wo_hbm, wo_v, 64)
        return ([p(ds(0, 7), 2 * j), p(ds(0, 7), 2 * j + 1)],
                [p(7, 2 * j), p(8, 2 * j + 2), p(7, 2 * j + 1), p(8, 2 * j + 3)])

    wq32, wuk32, wuv32 = (r.bitcast(jnp.uint32) for r in (wq_hbm, wuk_hbm, wuv_hbm))
    phases = [
        (16, nine_regions(wq32, wq_v, 32, 4)),
        (16, twelve_regions(0, (wuk32, wuk_v))),
        (16, twelve_regions(4)),
        (16, twelve_regions(16)),
        (16, twelve_regions(28, (wuv32, wuv_v))),
        (18, nine_regions(wg_hbm, wg_v, 64, 3)),
        (18, nine_regions(wu_hbm, wu_v, 64, 4)),
        (18, nine_regions(wd_hbm, wd_v, 64, 3)),
        (15, wo_regions),
    ]

    def copy(p, j, refs):
        return pltpu.make_async_copy(*refs, sems.at[(sum(n for n, _ in phases[:p]) + j) & (RING - 1)])

    def pause(n):
        def tick(_, c):
            v = pad_v[...]
            pad_v[...] = v * v
            return c
        lax.fori_loop(0, n, tick, 0)

    def wait(p, j, k):
        bulk, singles = phases[p][1](j)
        half = len(bulk) // 2
        for refs in (bulk[:half], bulk[half:], singles)[k]:
            copy(p, j, refs).wait()

    def start(p, j, early):
        bulk, singles = phases[p][1](j)
        if early:
            for refs in bulk:
                copy(p, j, refs).start(priority=1)
            pause(SHORT)
        for t, refs in enumerate(singles[:2] if early else singles[2:]):
            if t:
                pause(LONG)
            copy(p, j, refs).start()

    def start_ahead(p, j, early, j_min, j_max):
        n = phases[p][0]
        if j_max + AHEAD < n:
            start(p, j + AHEAD, early)
        elif j_min + AHEAD >= n:
            start(p + 1, j + AHEAD - n, early)
        else:
            pl.when(j + AHEAD < n)(lambda: start(p, j + AHEAD, early))
            pl.when(j + AHEAD >= n)(lambda: start(p + 1, j + AHEAD - n, early))

    def run(p, first, count, work=None, carry=None, shift=0, shift_max=0):
        def body(i, c):
            j = first + shift + i
            span = (first, first + shift_max + count - 1)
            wait(p, j, 0)
            start_ahead(p, j, True, *span)
            wait(p, j, 1)
            if work is not None:
                c = work(i, c)
            wait(p, j, 2)
            start_ahead(p, j, False, *span)
            return c
        return lax.fori_loop(0, count, body, carry)

    x_copy = pltpu.make_async_copy(x_hbm, x_v, xsem.at[0])
    wr_copy = pltpu.make_async_copy(wr_hbm, wr_v, xsem.at[1])
    for j in range(AHEAD):
        for refs in phases[0][1](j)[0]:
            copy(0, j, refs).start(priority=1)
    x_copy.start()
    wr_copy.start()
    pad_v[...] = jnp.zeros(pad_v.shape, F32)
    for j in range(AHEAD):
        for refs in phases[0][1](j)[1]:
            pause(LONG)
            copy(0, j, refs).start()

    run(0, 0, 1)
    x_copy.wait()
    wr_copy.wait()
    x = x_v[...].astype(F32)
    xc = x - jnp.mean(x, axis=-1, keepdims=True)
    var = jnp.mean(xc * xc, axis=-1, keepdims=True)
    xn_v[...] = (xc / jnp.sqrt(var + 1e-5)).astype(BF).astype(F32)

    def spread(group):
        n = _iota((128, 256), 1)
        e = _onehot(_iota((128, 256), 0) == n // (2 * group) * group + n % group)
        xn = xn_v[...]
        xn = jnp.concatenate([xn, xn], axis=0)
        xn = jnp.concatenate([xn, jnp.zeros((8, 64), F32)], axis=1).astype(BF)
        xe = jnp.concatenate([_dot(xn[:, i * 128:(i + 1) * 128], e) for i in range(5)], axis=1)[:, :2 * M]
        lhs_v[...] = jnp.where(_iota((8, 2 * M), 1) // group % 2 == _iota((8, 2 * M), 0) // 4, xe, 0.0)

    spread(1)
    run(0, 1, 15)

    def pair_rows(ref, j):
        w = [ref[r, ds(j, ref.shape[1] // NP, stride=NP), :] for r in range(ref.shape[0])]
        return pltpu.bitcast(jnp.concatenate(w, axis=0), BF)

    def q_proj(j, c):
        q_v[j] = _dot(lhs_v[...].astype(BF), pair_rows(wq_v, j))
        return c

    run(1, 0, NP, q_proj)

    def absorb(j, c):
        z = _dot_nt(q_v[j].astype(BF), pair_rows(wuk_v, j))
        keep = _iota((8, 2 * DC), 1) % 2 == _iota((8, 2 * DC), 0) // 4
        z_v[ds(_mult(j * 8, 8), 8), :] = jnp.where(keep, z * (D ** -0.5), 0.0)
        return c

    run(2, 0, NP, absorb)
    drop_e = _onehot(_iota((256, 128), 0) // 2 == _iota((256, 128), 1))
    for i in range(4):
        row_v[i] = _dot(z_v[:, i * 256:(i + 1) * 256].astype(BF), drop_e)
    for b in range(B):
        qb_v[b] = jnp.concatenate([row_v[i, ds(b, H, stride=B), :] for i in range(4)], axis=1).astype(BF)

    def scores(r, mx, half=None):
        if half is None:
            s = _dot_nt(qb_v[r >> 3], ckv_v[r])
            s_v[r, 0] = s[:, :256]
            s_v[r, 1] = s[:, 256:]
        else:
            s = _dot_nt(qb_v[r >> 3], ckv_v[r, ds(_mult(half * 256, 256), 256), :])
            s_v[r, half] = s
        for t in range(s.shape[1] // 128):
            mx = jnp.maximum(mx, s[:, t * 128:(t + 1) * 128])
        return mx

    def keep_max(b, mx):
        m_v[b] = jnp.broadcast_to(jnp.max(mx, axis=-1, keepdims=True), mx.shape)

    def values(r, c):
        l, acc = c
        m = m_v[r >> 3]
        p = [jnp.exp(s_v[r, t // 2, :, (t % 2) * 128:(t % 2 + 1) * 128] - m) for t in range(4)]
        l = l + ((p[0] + p[1]) + (p[2] + p[3]))
        return l, acc + _dot(jnp.concatenate(p, axis=1).astype(BF), ckv_v[r])

    def keep_context(b, c):
        out = c[1] / jnp.sum(c[0], axis=-1, keepdims=True)
        for i in range(4):
            row_v[i, ds(b, H, stride=B), :] = out[:, i * 128:(i + 1) * 128]

    mx0 = jnp.full((H, 128), -jnp.inf, F32)
    pv0 = (jnp.zeros((H, 128), F32), jnp.zeros((H, DC), F32))

    def first_scores(b, _):
        keep_max(b, run(3, 0, 8, lambda j, c: scores(8 * b + j, c), mx0, 8 * b, 8))

    lax.fori_loop(0, 2, first_scores, None)

    def first_values(b, mx):
        mx, pv = run(4, 0, 8, lambda j, c: (scores(16 + 4 * b + (j >> 1), c[0], j & 1), values(8 * b + j, c[1])),
                     (mx, pv0), 8 * b, 8)
        keep_context(b, pv)
        return mx

    keep_max(2, lax.fori_loop(0, 2, first_values, mx0))
    mx, pv = run(5, 0, 8, lambda j, c: (scores(24 + j, c[0]), values(16 + j, c[1])), (mx0, pv0))
    keep_context(2, pv)
    keep_max(3, mx)
    keep_context(3, run(5, 8, 8, lambda j, c: values(24 + j, c), pv0))
    run(5, 16, 1)
    add_e = _onehot(_iota((128, 256), 0) == _iota((128, 256), 1) // 2)
    keep = _iota((128, 256), 1) % 2 == (_iota((128, 256), 0) // 4) % 2
    for i in range(4):
        z_v[:, i * 256:(i + 1) * 256] = jnp.where(keep, _dot(row_v[i].astype(BF), add_e), 0.0)
    run(5, 17, 1)

    def up_v(j, c):
        ctx_v[j] = _dot(z_v[ds(_mult(j * 8, 8), 8), :].astype(BF), pair_rows(wuv_v, j))
        return c

    run(6, 0, NP, up_v)
    spread(8)
    so_v[...] = jnp.zeros(so_v.shape, F32)
    run(6, 16, 2)

    def tile_pair(ref, j, bands=range(8)):
        w = [ref[r, ds(_mult(band * 288 + j * 16, 16), 16), :] for r in range(9) for band in bands]
        return jnp.concatenate(w, axis=0)

    def gate_up(i, c):
        lhs = lhs_v[...].astype(BF)
        for j in (2 * i, 2 * i + 1):
            h_v[j] = jax.nn.silu(_dot(lhs, tile_pair(wg_v, j))) * _dot(lhs, tile_pair(wu_v, j))
        return c

    def down(js, bands, c):
        for j in js:
            c = c + _dot_nt(h_v[j].astype(BF), tile_pair(wd_v, j, bands))
        return c

    def out_proj(tiles):
        for r, j in tiles:
            tile = 16 * r + j
            pair = (tile * 57) >> 9
            so_v[tile - 9 * pair] += _dot_nt(ctx_v[pair].astype(BF), wo_v[r, ds(_mult(j * 128, 128), 128), :])

    first_tile = pltpu.make_async_copy(*part(wo_hbm, wo_v, 128, 8, 0), xsem.at[0])
    last_tiles = pltpu.make_async_copy(*part(wo_hbm, wo_v, 128, ds(0, 8), 15), xsem.at[1])
    first_tile.start(priority=1)
    run(7, 0, 9, gate_up)
    y0 = run(7, 9, 6, lambda i, c: down([3 * i + t for t in range(3)], range(4), c), jnp.zeros((8, M), F32))
    y1 = run(7, 15, 3, lambda i, c: down([6 * i + t for t in range(6)], (4, 5), c), jnp.zeros((8, M // 2), F32))
    first_tile.wait()
    out_proj([(8, 0)])

    last = len(phases) - 1
    late = 4 * (phases[last][0] - AHEAD)

    def last_rounds(first, count, work=None, carry=None):
        def body(i, c):
            def ahead():
                if first + AHEAD < phases[last][0]:
                    for refs in wo_regions(i + AHEAD)[0]:
                        copy(last, i + AHEAD, refs).start(priority=1)
                for k in range(3):
                    if k:
                        pause(LONG)
                    j, t = AHEAD + ((3 * i + k) >> 2), (3 * i + k) & 3
                    copy(last, j, part(wo_hbm, wo_v, 64, 7 + (t & 1), 2 * j + (t >> 1) + 2 * (t & 1))).start()

            wait(last, i, 0)
            if 3 * (first + count) <= late:
                ahead()
            else:
                pl.when(3 * i < late)(ahead)
            wait(last, i, 1)
            wait(last, i, 2)
            out_proj([(8, i + 1)] + [(r, i) for r in range(8)])
            return c if work is None else work(i, c)
        return lax.fori_loop(first, first + count, body, carry)

    y2 = last_rounds(0, 9, lambda i, c: down((2 * i, 2 * i + 1), (6, 7), c), jnp.zeros((8, M // 2), F32))
    last_tiles.start(priority=1)
    y0, y1, y2 = (jnp.concatenate([v, jnp.zeros((8, v.shape[1] // 9), F32)], axis=1) for v in (y0, y1, y2))
    yo = jnp.concatenate([v[:, i * n:(i + 1) * n] for i in range(5) for v, n in ((y0, 128), (y1, 64), (y2, 64))], axis=1)
    yo = jnp.where(_iota(yo.shape, 1) // 8 % 2 == _iota(yo.shape, 0) // 4, yo, 0.0)
    parts = []
    for _ in range(3):
        parts.append(yo.astype(BF).astype(F32))
        yo = yo - parts[-1]
    parts = jnp.concatenate(parts + [jnp.zeros_like(yo)], axis=0).astype(BF)
    n = _iota((256, 128), 0)
    region = jnp.where(n < 128, n // 64, n // 32 % 2)
    band = jnp.where(n < 128, n // 16 % 4, n // 64 * 2 + n // 16 % 2)
    in_order = _onehot(region * 64 + band * 8 + n % 8 == _iota((256, 128), 1))
    y = jnp.concatenate([_dot(parts[:, i * 256:(i + 1) * 256], in_order) for i in range(5)], axis=1)
    y = y[0:8] + y[8:16] + y[16:24]
    y = (y[0:4] + y[4:8])[:, :M]
    xn = xn_v[...]
    r = jnp.sum(xn * wr_v[...].astype(F32).reshape(1, M), axis=-1, keepdims=True)
    fin_v[...] = jnp.zeros(fin_v.shape, F32)
    fin_v[0, 0:4, 0:M] = jax.nn.silu(xn + (xn * 0.0 + y * jax.nn.sigmoid(r)))
    fin_v[1, 0:4, 0:M] = x_v[...].astype(F32)
    last_rounds(9, 6)

    low = _iota((8, 128), 1) < 64
    odd = [pltpu.roll(pltpu.roll(so_v[4 + t], 4, 0), 64, 1) for t in range(5)]
    s = [so_v[t] + jnp.where(low, odd[t], odd[min(t + 1, 4)]) for t in range(5)]
    starts = {r: divmod(2048 * r + 1920, M) for r in (1, 4, 5, 0, 2, 3, 6, 7)}
    lhs = {r: (pltpu.roll(ctx_v[head // 2], 4, 0) if head % 2 else ctx_v[head // 2]).astype(BF)
           for r, (head, _) in starts.items()}
    gate, x = ([fin_v[k, :, 128 * t:128 * (t + 1)] for t in range(5)] for k in range(2))
    last_tiles.wait()
    for r, (_, col) in starts.items():
        z = _dot_nt(lhs[r], wo_v[r, ds(1920, 128), :])
        if col == 512:
            s[4] += jnp.where(low, z, 0.0)
            s[0] += jnp.where(low, pltpu.roll(pltpu.roll(z, 4, 0), 64, 1), 0.0)
        elif col % 128 == 0:
            s[col // 128] += z
        else:
            z = pltpu.roll(z, 64, 1)
            s[col // 128] += jnp.where(low, 0.0, z)
            s[col // 128 + 1] += jnp.where(low, z, 0.0)
    for t in range(5):
        n = min(128, M - 128 * t)
        o_ref[:, 128 * t:128 * t + n] = (x[t] + s[t] * gate[t])[0:4, 0:n].astype(o_ref.dtype)


def _tiles(w):
    return w.reshape(72, 8, 36, 128).transpose(0, 2, 1, 3).reshape(9, 2304, 128)


@jax.jit
def pallas_recurrent_scan__compressed_kv_cla__moe_arch_mod__decode_kernel(
    A_x: jax.Array,
    A_c_kv: jax.Array,
    A_w_q: jax.Array,
    A_w_uk: jax.Array,
    A_w_uv: jax.Array,
    A_w_o: jax.Array,
    B_x: jax.Array,
    B_w_r: jax.Array,
    B_w_gate: jax.Array,
    B_w_up: jax.Array,
    B_w_down: jax.Array,
):
    del B_x
    out = pl.pallas_call(
        _kernel,
        out_shape=jax.ShapeDtypeStruct((B, M), A_x.dtype),
        in_specs=[pl.BlockSpec(memory_space=pltpu.HBM)] * 10,
        scratch_shapes=[
            pltpu.VMEM((B, M), BF),
            pltpu.VMEM((M,), BF),
            pltpu.VMEM((32, 512, DC), BF),
            pltpu.VMEM((9, 1024, D), jnp.uint32),
            pltpu.VMEM((8, 1024, D), jnp.uint32),
            pltpu.VMEM((8, 1024, D), jnp.uint32),
            pltpu.VMEM((9, 2048, D), BF),
            pltpu.VMEM((9, 2304, 128), BF),
            pltpu.VMEM((9, 2304, 128), BF),
            pltpu.VMEM((9, 2304, 128), BF),
            pltpu.VMEM((B, M), F32),
            pltpu.VMEM((8, 2 * M), F32),
            pltpu.VMEM((NP, 8, D), F32),
            pltpu.VMEM((B * H, 2 * DC), F32),
            pltpu.VMEM((4, B * H, 128), F32),
            pltpu.VMEM((B, H, DC), BF),
            pltpu.VMEM((32, 2, H, 256), F32),
            pltpu.VMEM((B, H, 128), F32),
            pltpu.VMEM((NP, 8, D), F32),
            pltpu.VMEM((F // 256, 8, 128), F32),
            pltpu.VMEM((9, 8, 128), F32),
            pltpu.VMEM((2, 8, 640), F32),
            pltpu.VMEM((8, 128), F32),
            pltpu.SemaphoreType.DMA((RING,)),
            pltpu.SemaphoreType.DMA((2,)),
        ],
        compiler_params=pltpu.CompilerParams(vmem_limit_bytes=100 * 1024 * 1024,
                                             disable_bounds_checks=True, disable_semaphore_checks=True),
    )(A_x.reshape(B, M), B_w_r, A_c_kv.reshape(32, 512, DC), A_w_q.reshape(9, 2048, D),
      A_w_uk.reshape(8, 2048, D), A_w_uv.reshape(8, 2048, D),
      jnp.transpose(A_w_o, (0, 2, 1)).reshape(9, 2048, D),
      _tiles(B_w_gate), _tiles(B_w_up), _tiles(B_w_down.T))
    return out.reshape(B, 1, M)
```
